```python
import os as _os
_os.environ.setdefault("JAX_PLATFORMS", "cpu")
import jax
import jax.numpy as jnp

def _softmax(x, axis=-1):
    return jax.nn.softmax(x, axis=axis)
def _gelu(x):
    return jax.nn.gelu(x, approximate=True)
def _silu(x):
    return jax.nn.silu(x)
def _sigmoid(x):
    return jax.nn.sigmoid(x)
def _layernorm(x, axis=-1, eps=1e-5):
    m = jnp.mean(x, axis=axis, keepdims=True)
    v = jnp.var(x, axis=axis, keepdims=True)
    return (x - m) / jnp.sqrt(v + eps)
def _scatter_add(tgt, idx, src, axis=0):
    return tgt.at[idx].add(src)
def _segment_sum(src, seg, n):
    return jax.ops.segment_sum(src, seg, n)
class _Rng:
    def __init__(self, key):
        self._k = key
    def _next(self):
        self._k, sub = jax.random.split(self._k)
        return sub
    def normal(self, shape):
        return jax.random.normal(self._next(), shape, dtype=jnp.bfloat16)
    def randint(self, lo, hi, shape):
        return jax.random.randint(self._next(), shape, lo, hi, dtype=jnp.int32)
    def uniform(self, shape, lo=0.0, hi=1.0):
        return jax.random.uniform(self._next(), shape, jnp.bfloat16, lo, hi)
    def permutation(self, n):
        return jax.random.permutation(self._next(), n)


kernel_name = 'standalone__dcn_v2_cross__recsys'

def setup_inputs():
    _rng = _Rng(jax.random.key(int.from_bytes(__import__("os").urandom(4), "little")))
    _w = (lambda a: (lambda t: t.astype(jnp.bfloat16) if jnp.issubdtype(t.dtype, jnp.floating) else t)(jnp.asarray(a)))
    B, F, D, L = 4096, 26, 128, 6
    Din = min(F * D, 1024)
    return {
        "x0": _w((lambda *s: _rng.normal(s) * 0.05)(B, Din)),
        "ws": _w((lambda *s: _rng.normal(s) * 0.05)(L, Din, Din)),
        "bs": _w((lambda *s: _rng.normal(s) * 0.05)(L, Din)),
    }

def reference(x0, ws, bs):
    x = x0
    for l in range(ws.shape[0]):
        x = x0 * (x @ ws[l] + bs[l]) + x
    return x
```

```python
import functools
import jax
import jax.numpy as jnp
from jax import lax
import jax.experimental.pallas as pl
import jax.experimental.pallas.tpu as pltpu

bf16 = jnp.bfloat16
f32 = jnp.float32


def make(tm=512):
    @jax.jit
    def fn(x0, ws, bs):
        B, D = x0.shape
        L = ws.shape[0]
        h = D // 2
        m = tm // 2
        n = B // tm

        def kernel(x0_hbm, w_hbm, b_hbm, o_hbm, w_raw, s_w, xbuf, obuf, xs_ref, b_raw, bf_ref, wsem, xsem, osem, bsem):
            def x_copy(i, slot):
                return pltpu.make_async_copy(x0_hbm.at[pl.ds(i * tm, tm)], xbuf.at[slot], xsem.at[slot])

            def o_copy(i, slot):
                return pltpu.make_async_copy(obuf.at[slot], o_hbm.at[pl.ds(i * tm, tm)], osem.at[slot])

            def w_copy(l):
                return pltpu.make_async_copy(w_hbm.at[l], w_raw.at[l], wsem.at[l])

            b_copy = pltpu.make_async_copy(b_hbm, b_raw, bsem.at[0])

            copies = [b_copy, x_copy(0, 0)] + [w_copy(l) for l in range(L)]
            if n > 1:
                copies.append(x_copy(1, 1))

            def issue(j, carry):
                for idx, cp in enumerate(copies):
                    @pl.when(j == idx)
                    def _(cp=cp):
                        cp.start()
                return carry

            lax.fori_loop(0, len(copies), issue, 0)

            def dot(a, w):
                return jnp.dot(a.astype(bf16), w, preferred_element_type=f32)

            def layer(l, A, X, first):
                A11, A12, A21, A22 = A
                X11, X12, X21, X22 = X
                b1 = bf_ref[l, :, :h]
                b2 = bf_ref[l, :, h:]
                B11 = w_raw[l, :h, :h]
                B22 = w_raw[l, h:, h:]
                if first:
                    M5 = dot(A11 + A12, B22)
                    M2 = dot(A21 + A22, B11)
                    B11f = B11.astype(f32)
                    B22f = B22.astype(f32)
                    B12f = w_raw[l, :h, h:].astype(f32)
                    B21f = w_raw[l, h:, :h].astype(f32)
                    S3 = (B12f - B22f).astype(bf16)
                    S4 = (B21f - B11f).astype(bf16)
                    S1 = (B11f + B22f).astype(bf16)
                    S7 = (B21f + B22f).astype(bf16)
                    S6 = (B11f + B12f).astype(bf16)
                    s_w[l, 0] = S3
                    s_w[l, 1] = S4
                    s_w[l, 2] = S1
                    s_w[l, 3] = S7
                    s_w[l, 4] = S6
                    M3 = dot(A11, S3)
                    N12 = X12 * (M3 + M5 + b2) + A12
                    M4 = dot(A22, S4)
                    N21 = X21 * (M2 + M4 + b1) + A21
                    M1 = dot(A11 + A22, S1)
                    M7 = dot(A12 - A22, S7)
                    N11 = X11 * (M1 + M4 - M5 + M7 + b1) + A11
                    M6 = dot(A21 - A11, S6)
                    N22 = X22 * (M1 - M2 + M3 + M6 + b2) + A22
                else:
                    M3 = dot(A11, s_w[l, 0])
                    M5 = dot(A11 + A12, B22)
                    N12 = X12 * (M3 + M5 + b2) + A12
                    M2 = dot(A21 + A22, B11)
                    M4 = dot(A22, s_w[l, 1])
                    N21 = X21 * (M2 + M4 + b1) + A21
                    M1 = dot(A11 + A22, s_w[l, 2])
                    M7 = dot(A12 - A22, s_w[l, 3])
                    N11 = X11 * (M1 + M4 - M5 + M7 + b1) + A11
                    M6 = dot(A21 - A11, s_w[l, 4])
                    N22 = X22 * (M1 - M2 + M3 + M6 + b2) + A22
                return N11, N12, N21, N22

            quads = [(slice(0, m), slice(0, h)), (slice(0, m), slice(h, D)),
                     (slice(m, tm), slice(0, h)), (slice(m, tm), slice(h, D))]

            b_copy.wait()
            bb = b_raw[...].astype(f32)
            for l in range(L):
                bf_ref[l] = bb[l:l + 1, :]
            x_copy(0, 0).wait()
            xs_ref[...] = xbuf[0].astype(f32)

            def first_body(l, carry):
                w_copy(l).wait()
                A = [xs_ref[r, c] for r, c in quads]
                X = [xbuf[0, r, c].astype(f32) for r, c in quads]
                N = layer(l, A, X, True)
                for (r, c), v in zip(quads, N):
                    xs_ref[r, c] = v
                return carry

            lax.fori_loop(0, L, first_body, 0)
            obuf[0] = xs_ref[...].astype(bf16)
            o_copy(0, 0).start()

            def step(i, carry):
                slot = i % 2
                x_copy(i, slot).wait()

                @pl.when(i + 1 < n)
                def _():
                    x_copy(i + 1, 1 - slot).start()

                @pl.when(i >= 2)
                def _():
                    o_copy(i - 2, slot).wait()

                X = [xbuf[slot, r, c].astype(f32) for r, c in quads]
                A = X
                for l in range(L):
                    A = layer(l, A, X, False)
                for (r, c), v in zip(quads, A):
                    obuf[slot, r, c] = v.astype(bf16)
                o_copy(i, slot).start()
                return carry

            lax.fori_loop(1, n, step, 0)
            if n > 1:
                o_copy(n - 2, (n - 2) % 2).wait()
            o_copy(n - 1, (n - 1) % 2).wait()

        return pl.pallas_call(
            kernel,
            in_specs=[pl.BlockSpec(memory_space=pl.ANY)] * 3,
            out_specs=pl.BlockSpec(memory_space=pl.ANY),
            out_shape=jax.ShapeDtypeStruct((B, D), x0.dtype),
            scratch_shapes=[
                pltpu.VMEM((L, D, D), bf16),
                pltpu.VMEM((L, 5, h, h), bf16),
                pltpu.VMEM((2, tm, D), bf16),
                pltpu.VMEM((2, tm, D), bf16),
                pltpu.VMEM((tm, D), f32),
                pltpu.VMEM((L, D), bf16),
                pltpu.VMEM((L, 1, D), f32),
                pltpu.SemaphoreType.DMA((L,)),
                pltpu.SemaphoreType.DMA((2,)),
                pltpu.SemaphoreType.DMA((2,)),
                pltpu.SemaphoreType.DMA((1,)),
            ],
            compiler_params=pltpu.CompilerParams(
                vmem_limit_bytes=100 * 1024 * 1024,
            ),
        )(x0, ws, bs)
    return fn


pallas_standalone__dcn_v2_cross__recsys_kernel = make(512)
```

```python
import functools
import jax
import jax.numpy as jnp
from jax import lax
import jax.experimental.pallas as pl
import jax.experimental.pallas.tpu as pltpu

bf16 = jnp.bfloat16
f32 = jnp.float32

A_OPS = {0: ((0, 1), (3, 1)), 1: ((2, 1), (3, 1)), 2: ((0, 1),), 3: ((3, 1),),
         4: ((0, 1), (1, 1)), 5: ((2, 1), (0, -1)), 6: ((1, 1), (3, -1))}
B_OPS = {0: ((0, 1), (3, 1)), 1: ((0, 1),), 2: ((1, 1), (3, -1)), 3: ((2, 1), (0, -1)),
         4: ((3, 1),), 5: ((0, 1), (1, 1)), 6: ((2, 1), (3, 1))}


def _split(a):
    r, c = a.shape[0] // 2, a.shape[1] // 2
    return a[:r, :c], a[:r, c:], a[r:, :c], a[r:, c:]


def _join(c11, c12, c21, c22):
    return jnp.concatenate([jnp.concatenate([c11, c12], axis=1),
                            jnp.concatenate([c21, c22], axis=1)], axis=0)


def _lin(terms):
    terms = sorted(terms, key=lambda t: -t[1])
    acc = terms[0][0]
    for v, s in terms[1:]:
        acc = acc + v if s > 0 else acc - v
    return acc


def _lin2(get, o1, o2):
    if len(o1) == 2 and len(o2) == 2:
        t = lambda i, k: (get(o1[i][0], o2[k][0]), o1[i][1] * o2[k][1])
        p1, p2 = [t(0, 0), t(1, 1)], [t(0, 1), t(1, 0)]
        if p2[0][1] > 0 or p2[1][1] > 0:
            return _lin(p1) + _lin(p2)
        return _lin(p1) - _lin([(v, -s) for v, s in p2])
    return _lin([(get(q, q2), s * s2) for q, s in o1 for q2, s2 in o2])


def _chain(mul, acc, same):
    if acc is None:
        r1 = mul(3, None)
        r2 = mul(1, r1)
        r3 = mul(0, r1 - r2)
        r4 = mul(5, r3)
        r5 = mul(2, r4)
        f = r5 - r4
        r6 = mul(4, f)
        r7 = mul(6, (r3 + r2) + (f - r6))
        return r7, r6, r2, r5
    a11, a12, a21, a22 = acc
    r1 = mul(3, a21)
    r2 = mul(1, r1)
    r3 = mul(0, r1 - r2)
    if same:
        r4 = mul(5, r3)
        r5 = mul(2, r4 + a22)
        f = r5 - r4
        r6 = mul(4, f)
        r7 = mul(6, (r3 + r2) + (f - r6))
    else:
        r4 = mul(5, r3 + a22)
        r5 = mul(2, r4)
        f = (r5 - r4) + a12
        r6 = mul(4, f)
        r7 = mul(6, ((r3 + r2) + (a11 - a21)) + (f - r6))
    return r7, r6, r2, r5


def make(tm=512, deep=(1, 2, 3, 4, 5, 6), swap=(1, 2, 3, 4), guard=True, tx=7.0, tw=6.5, fchain=False,
         wsub=32, wacc=1, xmode='max', xacc=4, wsteady=True, gmax=1.0):
    deep = tuple(deep)
    s1_slot = {j: i for i, j in enumerate(j for j in range(7) if j not in deep and len(B_OPS[j]) > 1)}
    s2_slot = {k: i for i, k in enumerate((j, j2) for j in deep for j2 in range(7)
                                          if len(B_OPS[j]) * len(B_OPS[j2]) > 1)}
    stat_leaves = [(j, j2) for j in (2, 3, 5, 6) for j2 in (1, 4)]

    @jax.jit
    def fn(x0, ws, bs):
        B, D = x0.shape
        L = ws.shape[0]
        h = D // 2
        g = D // 4
        m = tm // 2
        n = B // tm
        sc = 128
        nc = D // 128

        def kernel(x0_hbm, w_hbm, b_hbm, o_hbm, w_raw, s1_w, s2_w, xbuf, obuf, xs_ref, b_raw, bf_ref,
                   wsem, xsem, osem, psem):
            lo, hi = slice(0, h), slice(h, D)
            top, bot = slice(0, m), slice(m, tm)
            quads = [(top, lo), (top, hi), (bot, lo), (bot, hi)]
            wq = [(lo, lo), (lo, hi), (hi, lo), (hi, hi)]

            def x_copy(i, slot):
                return pltpu.make_async_copy(x0_hbm.at[pl.ds(i * tm, tm)], xbuf.at[slot], xsem.at[slot])

            def o_copies(i, slot):
                return [pltpu.make_async_copy(obuf.at[slot, r, c],
                                              o_hbm.at[pl.ds(i * tm + r.start, m), c],
                                              osem.at[slot * 4 + q]) for q, (r, c) in enumerate(quads)]

            def w_copy(l):
                return pltpu.make_async_copy(w_hbm.at[l], w_raw.at[l], wsem.at[l])

            b_copy = pltpu.make_async_copy(b_hbm, b_raw, psem.at[0])
            wq_copy = [pltpu.make_async_copy(w_hbm.at[(0,) + wq[q]], w_raw.at[(0,) + wq[q]], psem.at[1 + q])
                       for q in range(4)]
            xt_copy = pltpu.make_async_copy(x0_hbm.at[top], xbuf.at[0, top], psem.at[5])
            xb_copy = pltpu.make_async_copy(x0_hbm.at[bot], xbuf.at[0, bot], psem.at[6])

            copies = [xt_copy, wq_copy[3], b_copy, xb_copy, wq_copy[0], wq_copy[1], wq_copy[2]]
            copies += [w_copy(l) for l in range(1, L)]
            if n > 1:
                copies.append(x_copy(1, 1))

            def issue(j, carry):
                for idx, cp in enumerate(copies):
                    @pl.when(j == idx)
                    def _(cp=cp):
                        cp.start()
                return carry

            lax.fori_loop(0, len(copies), issue, 0)

            def dot(a, w):
                return jnp.dot(a.astype(bf16), w, preferred_element_type=f32)

            pk = lambda v: pltpu.bitcast(v, jnp.uint32)
            upk = lambda v: pltpu.bitcast(v, bf16)

            def raw_sub(l, j, q, q2):
                c2 = (q2 % 2) ^ (1 if j in swap else 0)
                rr = (q // 2) * h + (q2 // 2) * g
                cc = (q % 2) * h + c2 * g
                return w_raw[l, rr:rr + g, cc:cc + g]

            def product(l, j, geta, acc, build, isbias=False):
                if j in deep:
                    sub = lambda q, q2: _split(geta(q))[q2]
                    if build and len(B_OPS[j]) > 1:
                        V = [_lin([(raw_sub(l, j, q, q2).astype(f32), s) for q, s in B_OPS[j]])
                             for q2 in range(4)]

                    def mul2(j2, acc2):
                        o1, o2 = A_OPS[j], A_OPS[j2]
                        if len(o1) * len(o2) == 1:
                            a2 = sub(o1[0][0], o2[0][0])
                        else:
                            a2 = _lin2(lambda q, q2: sub(q, q2).astype(f32), o1, o2)
                        if (j, j2) not in s2_slot:
                            w = raw_sub(l, j, B_OPS[j][0][0], B_OPS[j2][0][0])
                        elif not build:
                            w = upk(s2_w[l, s2_slot[j, j2]])
                        else:
                            if len(B_OPS[j]) > 1:
                                wf = _lin([(V[q2], s) for q2, s in B_OPS[j2]])
                            else:
                                wf = _lin([(raw_sub(l, j, B_OPS[j][0][0], q2).astype(f32), s)
                                           for q2, s in B_OPS[j2]])
                            w = wf.astype(bf16)
                            s2_w[l, s2_slot[j, j2]] = pk(w)
                        r = dot(a2, w)
                        return r if acc2 is None else r + acc2

                    a = None if acc is None else _split(acc)
                    if j in swap:
                        c = _chain(mul2, None if a is None else (a[1], a[0], a[3], a[2]), isbias)
                        return _join(c[1], c[0], c[3], c[2])
                    return _join(*_chain(mul2, a, isbias))
                if len(A_OPS[j]) == 1:
                    a = geta(A_OPS[j][0][0])
                else:
                    a = _lin([(geta(q).astype(f32), s) for q, s in A_OPS[j]])
                if len(B_OPS[j]) == 1:
                    w = w_raw[(l,) + wq[B_OPS[j][0][0]]]
                elif not build:
                    w = upk(s1_w[l, s1_slot[j]])
                else:
                    w = _lin([(w_raw[(l,) + wq[q]].astype(f32), s) for q, s in B_OPS[j]]).astype(bf16)
                    s1_w[l, s1_slot[j]] = pk(w)
                r = dot(a, w)
                return r if acc is None else r + acc

            def bias(l, rows):
                bv = bf_ref[l]
                return (jnp.broadcast_to(bv[:, lo], (rows, h)), jnp.broadcast_to(bv[:, hi], (rows, h)))

            def x_stats(parts, ssv, maxv):
                ssv = list(ssv)
                for blk, c0 in parts:
                    for c in range(blk.shape[1] // 128):
                        ss, mx = None, None
                        for r in range(0, blk.shape[0], 8):
                            t = blk[r:r + 8, c * 128:(c + 1) * 128]
                            t = t * t
                            ss = t if ss is None else ss + t
                            mx = t if mx is None else jnp.maximum(mx, t)
                        ssv[c0 + c] = ss if ssv[c0 + c] is None else ssv[c0 + c] + ss
                        maxv = mx if maxv is None else jnp.maximum(maxv, mx)
                return tuple(ssv), maxv

            def w_partials(l):
                mh, ml, ss = [None] * wacc, [None] * wacc, None
                k = 0
                for key in stat_leaves:
                    wv = pltpu.bitcast(s2_w[l, s2_slot[key]], jnp.int32)
                    for r in range(0, g // 2, 8):
                        for c in range(0, g, 128):
                            u = wv[r:r + 8, c:c + 128] & jnp.int32(0x7FFF7FFF)
                            ul = pltpu.bitcast(u << 16, f32)
                            u = pltpu.bitcast(u, f32)
                            a = k % wacc
                            k += 1
                            mh[a] = u if mh[a] is None else jnp.maximum(mh[a], u)
                            ml[a] = ul if ml[a] is None else jnp.maximum(ml[a], ul)
                            if 2 * r < wsub:
                                s2 = ul * ul
                                ss = s2 if ss is None else ss + s2
                return functools.reduce(jnp.maximum, mh + ml), ss

            x_q = lambda q: xbuf[(0,) + quads[q]]
            ssv, maxv = (None,) * nc, None
            xt_copy.wait()
            if guard:
                ssv, maxv = x_stats([(xbuf[0, top].astype(f32), 0)], ssv, maxv)
            wq_copy[3].wait()
            M5 = product(0, 4, x_q, None, True)
            b_copy.wait()
            xb_copy.wait()
            bb = b_raw[...].astype(f32)
            for k in range(L):
                bf_ref[k] = bb[k:k + 1, :]
            if guard:
                ssv, maxv = x_stats([(xbuf[0, bot].astype(f32), 0)], ssv, maxv)
            else:
                ssv, maxv = (jnp.zeros((8, 128), f32),) * nc, jnp.zeros((8, 128), f32)
            wq_copy[0].wait()
            M2 = product(0, 1, x_q, None, True)
            M1 = product(0, 0, x_q, None, True)
            wq_copy[1].wait()
            wq_copy[2].wait()
            b1, b2 = bias(0, m)
            M3b = product(0, 2, x_q, b2, True, True)
            M4b = product(0, 3, x_q, b1, True, True)
            C11 = product(0, 6, x_q, M1 + M4b - M5, True)
            C22 = product(0, 5, x_q, M1 + M3b - M2, True)
            for q, C in enumerate((C11, M3b + M5, M2 + M4b, C22)):
                a = x_q(q).astype(f32)
                xs_ref[quads[q]] = a * C + a

            def first_body(l, carry):
                w_copy(l).wait()
                A = [xs_ref[quads[q]] for q in range(4)]
                geta = lambda q: A[q]
                b1, b2 = bias(l, m)
                if fchain:
                    Cs = _chain(lambda j, acc: product(l, j, geta, acc, True, j == 3), (b1, b2, b1, b2), True)
                else:
                    M5 = product(l, 4, geta, None, True)
                    M2 = product(l, 1, geta, None, True)
                    M3b = product(l, 2, geta, b2, True, True)
                    M4b = product(l, 3, geta, b1, True, True)
                    M1 = product(l, 0, geta, None, True)
                    C11 = product(l, 6, geta, M1 + M4b - M5, True)
                    C22 = product(l, 5, geta, M1 + M3b - M2, True)
                    Cs = (C11, M3b + M5, M2 + M4b, C22)
                for q, C in enumerate(Cs):
                    xs_ref[quads[q]] = x_q(q).astype(f32) * C + A[q]
                return carry

            lax.fori_loop(1, L, first_body, 0)
            obuf[0] = xs_ref[...].astype(bf16)
            for cp in o_copies(0, 0):
                cp.start()

            def step(i, carry):
                ssv, maxv = carry
                slot = i % 2

                @pl.when(i + 1 < n)
                def _():
                    x_copy(i + 1, 1 - slot).start()

                x_copy(i, slot).wait()

                @pl.when(i >= 2)
                def _():
                    for cp in o_copies(i - 2, slot):
                        cp.wait()

                Xb = [xbuf[(slot,) + quads[q]] for q in range(4)]
                X = [v.astype(f32) for v in Xb]
                if guard and xmode == 'full':
                    ssv, maxv = x_stats([(jnp.concatenate([X[0], X[2]], axis=0), 0),
                                         (jnp.concatenate([X[1], X[3]], axis=0), nc // 2)], ssv, maxv)
                elif guard:
                    acc = [None] * xacc
                    k = 0
                    for blk in X:
                        for c in range(0, h, 128):
                            for r in range(0, m, 8):
                                t = jnp.abs(blk[r:r + 8, c:c + 128])
                                a = (k * xacc) // (4 * (h // 128) * (m // 8))
                                k += 1
                                acc[a] = t if acc[a] is None else jnp.maximum(acc[a], t)
                    t = functools.reduce(jnp.maximum, acc)
                    maxv = jnp.maximum(maxv, t * t)
                    if wsteady:
                        lw = jnp.minimum(i - 1, L - 1)
                        pm, ps = w_partials(lw)
                        ssv = tuple((jnp.where(lw == k, pm, a), jnp.where(lw == k, ps, b))
                                    for k, (a, b) in enumerate(ssv))
                A = X
                for l in range(L):
                    src = Xb if l == 0 else A
                    b1, b2 = bias(l, m)
                    C = _chain(lambda j, acc: product(l, j, lambda q: src[q], acc, False, j == 3),
                               (b1, b2, b1, b2), True)
                    A = [x * c + a for x, c, a in zip(X, C, A)]
                ocs = o_copies(i, slot)
                for q in (2, 3, 1, 0):
                    obuf[(slot,) + quads[q]] = A[q].astype(bf16)
                    ocs[q].start()
                return ssv, maxv

            if xmode == 'full':
                ssv, maxv = lax.fori_loop(1, n, step, (ssv, maxv))
            else:
                z = jnp.zeros((8, 128), f32)
                wcar, maxv = lax.fori_loop(1, n, step, (((z, z),) * L if wsteady else (), maxv))

            if guard:
                def unsafe(mx, ms, t):
                    ok = jnp.logical_and(mx <= (t * t) * ms, jnp.logical_and(mx < 1e30, ms > 1e-30))
                    return jnp.where(ok, 0, 1).astype(jnp.int32)

                cols = functools.reduce(jnp.minimum, [jnp.sum(v, axis=0, keepdims=True) for v in ssv])
                mx_x = jnp.max(maxv)
                bad = unsafe(mx_x, jnp.min(cols) * (1.0 / (B if xmode == 'full' else tm)), tx)
                gain = 0.0
                for l in range(L):
                    mxv, ssw = wcar[l] if wsteady else w_partials(l)
                    mx = jnp.max(mxv)
                    ms = jnp.sum(ssw) * (2.0 / (len(stat_leaves) * wsub * g))
                    bad = bad + unsafe(mx * mx, ms, tw)
                    gain = gain + jnp.minimum((0.5 * D) * mx_x * ms, 1.0)
                bad = bad + jnp.where(gain <= gmax, 0, 1).astype(jnp.int32)

            for t in (n - 2, n - 1):
                for cp in o_copies(t, t % 2):
                    cp.wait()

            if guard:
                @pl.when(bad > 0)
                def _():
                    def redo(i, carry):
                        x_copy(i, 0).start()
                        x_copy(i, 0).wait()

                        def body(t, carry):
                            c = t // L
                            l = t % L
                            rows = pl.ds(pl.multiple_of(c * sc, sc), sc)
                            x0c = xbuf[0, rows, :].astype(f32)
                            x = jnp.where(l == 0, x0c, xs_ref[rows, :])
                            xn = x0c * (dot(x, w_raw[l]) + bf_ref[l]) + x
                            xs_ref[rows, :] = xn
                            obuf[0, rows, :] = xn.astype(bf16)
                            return carry

                        lax.fori_loop(0, (tm // sc) * L, body, 0)
                        for cp in o_copies(i, 0):
                            cp.start()
                        for cp in o_copies(i, 0):
                            cp.wait()
                        return carry

                    lax.fori_loop(0, n, redo, 0)

        return pl.pallas_call(
            kernel,
            in_specs=[pl.BlockSpec(memory_space=pl.ANY)] * 3,
            out_specs=pl.BlockSpec(memory_space=pl.ANY),
            out_shape=jax.ShapeDtypeStruct((B, D), x0.dtype),
            scratch_shapes=[
                pltpu.VMEM((L, D, D), bf16),
                pltpu.VMEM((L, max(len(s1_slot), 1), h // 2, h), jnp.uint32),
                pltpu.VMEM((L, max(len(s2_slot), 1), g // 2, g), jnp.uint32),
                pltpu.VMEM((2, tm, D), bf16),
                pltpu.VMEM((2, tm, D), bf16),
                pltpu.VMEM((tm, D), f32),
                pltpu.VMEM((L, D), bf16),
                pltpu.VMEM((L, 1, D), f32),
                pltpu.SemaphoreType.DMA((L,)),
                pltpu.SemaphoreType.DMA((2,)),
                pltpu.SemaphoreType.DMA((8,)),
                pltpu.SemaphoreType.DMA((8,)),
            ],
            compiler_params=pltpu.CompilerParams(
                vmem_limit_bytes=120 * 1024 * 1024,
                disable_bounds_checks=True,
            ),
        )(x0, ws, bs)
    return fn


pallas_standalone__dcn_v2_cross__recsys_kernel = make(deep=(0, 1, 2, 3, 4, 5, 6), swap=(0, 2, 3))
```

```python
import functools

import jax
import jax.numpy as jnp
from jax import lax
import jax.experimental.pallas as pl
import jax.experimental.pallas.tpu as pltpu

bf16 = jnp.bfloat16
f32 = jnp.float32

_A_OPS = {0: ((0, 1), (3, 1)), 1: ((2, 1), (3, 1)), 2: ((0, 1),), 3: ((3, 1),),
          4: ((0, 1), (1, 1)), 5: ((2, 1), (0, -1)), 6: ((1, 1), (3, -1))}
_B_OPS = {0: ((0, 1), (3, 1)), 1: ((0, 1),), 2: ((1, 1), (3, -1)), 3: ((2, 1), (0, -1)),
          4: ((3, 1),), 5: ((0, 1), (1, 1)), 6: ((2, 1), (3, 1))}
_SWAP = (0, 2, 3)
_SLOT = {k: i for i, k in enumerate((j, j2) for j in range(7) for j2 in range(7)
                                    if len(_B_OPS[j]) * len(_B_OPS[j2]) > 1)}
_STAT_LEAVES = [(j, j2) for j in (2, 3, 5, 6) for j2 in (1, 4)]

_TM0 = 640
_TM = 576
_SC = 128
_WSUB = 32
_TX = 7.0
_TW = 6.5
_GMAX = 2.0


def _split(a):
    r, c = a.shape[0] // 2, a.shape[1] // 2
    return a[:r, :c], a[:r, c:], a[r:, :c], a[r:, c:]


def _join(c11, c12, c21, c22):
    return jnp.concatenate([jnp.concatenate([c11, c12], axis=1),
                            jnp.concatenate([c21, c22], axis=1)], axis=0)


def _lin(terms):
    terms = sorted(terms, key=lambda t: -t[1])
    acc = terms[0][0]
    for v, s in terms[1:]:
        acc = acc + v if s > 0 else acc - v
    return acc


def _lin2(get, o1, o2):
    if len(o1) == 2 and len(o2) == 2:
        t = lambda i, k: (get(o1[i][0], o2[k][0]), o1[i][1] * o2[k][1])
        p1, p2 = [t(0, 0), t(1, 1)], [t(0, 1), t(1, 0)]
        if p2[0][1] > 0 or p2[1][1] > 0:
            return _lin(p1) + _lin(p2)
        return _lin(p1) - _lin([(v, -s) for v, s in p2])
    return _lin([(get(q, q2), s * s2) for q, s in o1 for q2, s2 in o2])


def _chain(mul, acc, same, alt=False):
    a11, a12, a21, a22 = (None,) * 4 if acc is None else acc
    if alt:
        r1 = mul(1, a21)
        r2 = mul(3, r1)
        r3 = mul(0, -r1 if a21 is None else a21 - r1)
    else:
        r1 = mul(3, a21)
        r2 = mul(1, r1)
        r3 = mul(0, r1 - r2)
    if acc is None:
        r4 = mul(5, r3)
        r5 = mul(2, r4)
        f = r5 - r4
        r6 = mul(4, f)
        r7 = mul(6, (r3 + r2) + (f - r6))
    elif same:
        r4 = mul(5, r3)
        r5 = mul(2, r4 + a22)
        f = r5 - r4
        r6 = mul(4, f)
        r7 = mul(6, (r3 + r2) + (f - r6))
    else:
        r4 = mul(5, r3 + a22)
        r5 = mul(2, r4)
        f = (r5 - r4) + a12
        r6 = mul(4, f)
        r7 = mul(6, ((r3 + r2) + (a11 - a21)) + (f - r6))
    return r7, r6, r2, r5


@jax.jit
def pallas_standalone__dcn_v2_cross__recsys_kernel(
    x0: jax.Array,
    ws: jax.Array,
    bs: jax.Array,
):
    B, D = x0.shape
    L = ws.shape[0]
    tm0, tm, sc = _TM0, _TM, _SC
    h, g, nc = D // 2, D // 4, D // 128
    n = (B - tm0) // tm
    assert tm0 + n * tm == B and n >= max(L, 2) and B % sc == 0 and D % 512 == 0
    m0, m = tm0 // 2, tm // 2

    def kernel(x0_hbm, w_hbm, b_hbm, o_hbm, w_raw, s2_w, xbuf, obuf, xs_ref, b_raw, bf_ref,
               wsem, xsem, osem, psem):
        lo, hi = slice(0, h), slice(h, D)
        wq = [(lo, lo), (lo, hi), (hi, lo), (hi, hi)]

        def quads_of(t):
            top, bot = slice(0, t // 2), slice(t // 2, t)
            return [(top, lo), (top, hi), (bot, lo), (bot, hi)]

        quads0, quads = quads_of(tm0), quads_of(tm)
        top0, bot0 = slice(0, m0), slice(m0, tm0)

        def x_copy(i, slot):
            return pltpu.make_async_copy(x0_hbm.at[pl.ds(tm0 + i * tm, tm)],
                                         xbuf.at[slot, pl.ds(0, tm)], xsem.at[slot])

        def pieces(qs):
            r, c = qs[0]
            rm, cm = (r.start + r.stop) // 2, (c.start + c.stop) // 2
            rt, rb, cl, cr = slice(r.start, rm), slice(rm, r.stop), slice(c.start, cm), slice(cm, c.stop)
            return [qs[2], qs[3], qs[1], (rb, cl), (rb, cr), (rt, cr), (rt, cl)]

        def o_copies(row0, slot):
            return [pltpu.make_async_copy(obuf.at[slot, r, c],
                                          o_hbm.at[pl.ds(row0 + r.start, r.stop - r.start), c],
                                          osem.at[slot]) for r, c in pieces(quads)]

        def o_wait(rows, slot):
            v = obuf.at[slot, pl.ds(0, rows)]
            pltpu.make_async_copy(v, v, osem.at[slot]).wait()

        def w_copy(l):
            return pltpu.make_async_copy(w_hbm.at[l], w_raw.at[l], wsem.at[l])

        b_copy = pltpu.make_async_copy(b_hbm, b_raw, psem.at[0])
        wq_copy = [pltpu.make_async_copy(w_hbm.at[(0,) + wq[q]], w_raw.at[(0,) + wq[q]], psem.at[1 + q])
                   for q in range(4)]
        xt_copy = pltpu.make_async_copy(x0_hbm.at[top0], xbuf.at[1, top0], psem.at[5])
        xb_copy = pltpu.make_async_copy(x0_hbm.at[bot0], xbuf.at[1, bot0], psem.at[6])

        copies = [xt_copy, wq_copy[3], b_copy, xb_copy, wq_copy[0], wq_copy[1], wq_copy[2]]
        copies += [w_copy(l) for l in range(1, L)] + [x_copy(0, 0)]

        def issue(k, carry):
            for idx, cp in enumerate(copies):
                @pl.when(k == idx)
                def _(cp=cp):
                    cp.start()
            return carry

        lax.fori_loop(0, len(copies), issue, 0)

        def dot(a, w):
            return jnp.dot(a.astype(bf16), w, preferred_element_type=f32)

        def raw_sub(l, j, q, q2):
            c2 = (q2 % 2) ^ (1 if j in _SWAP else 0)
            rr = (q // 2) * h + (q2 // 2) * g
            cc = (q % 2) * h + c2 * g
            return w_raw[l, rr:rr + g, cc:cc + g]

        def product(l, j, geta, acc, build, isbias=False):
            sub = lambda q, q2: _split(geta(q))[q2]
            if build and len(_B_OPS[j]) > 1:
                V = [_lin([(raw_sub(l, j, q, q2).astype(f32), s) for q, s in _B_OPS[j]])
                     for q2 in range(4)]

            def mul2(j2, acc2):
                o1, o2 = _A_OPS[j], _A_OPS[j2]
                if len(o1) * len(o2) == 1:
                    a2 = sub(o1[0][0], o2[0][0])
                else:
                    a2 = _lin2(lambda q, q2: sub(q, q2).astype(f32), o1, o2)
                if (j, j2) not in _SLOT:
                    w = raw_sub(l, j, _B_OPS[j][0][0], _B_OPS[j2][0][0])
                elif not build:
                    w = pltpu.bitcast(s2_w[l, _SLOT[j, j2]], bf16)
                else:
                    if len(_B_OPS[j]) > 1:
                        wf = _lin([(V[q2], s) for q2, s in _B_OPS[j2]])
                    else:
                        wf = _lin([(raw_sub(l, j, _B_OPS[j][0][0], q2).astype(f32), s)
                                   for q2, s in _B_OPS[j2]])
                    w = wf.astype(bf16)
                    s2_w[l, _SLOT[j, j2]] = pltpu.bitcast(w, jnp.uint32)
                r = dot(a2, w)
                return r if acc2 is None else r + acc2

            a = None if acc is None else _split(acc)
            if j in _SWAP:
                c = _chain(mul2, None if a is None else (a[1], a[0], a[3], a[2]), isbias, build)
                return _join(c[1], c[0], c[3], c[2])
            return _join(*_chain(mul2, a, isbias, build))

        def bias(l, rows):
            bv = bf_ref[l]
            return jnp.broadcast_to(bv[:, lo], (rows, h)), jnp.broadcast_to(bv[:, hi], (rows, h))

        def x_stats(blk, ssv, maxv):
            ssv = list(ssv)
            for c in range(nc):
                ss = mx = None
                for r in range(0, blk.shape[0], 8):
                    t = blk[r:r + 8, c * 128:(c + 1) * 128]
                    t = t * t
                    ss = t if ss is None else ss + t
                    mx = t if mx is None else jnp.maximum(mx, t)
                ssv[c] = ss if ssv[c] is None else ssv[c] + ss
                maxv = mx if maxv is None else jnp.maximum(maxv, mx)
            return tuple(ssv), maxv

        def w_stats(l):
            mh = ml = ss = None
            for key in _STAT_LEAVES:
                wv = pltpu.bitcast(s2_w[l, _SLOT[key]], jnp.int32)
                for r in range(0, g // 2, 8):
                    for c in range(0, g, 128):
                        u = wv[r:r + 8, c:c + 128] & jnp.int32(0x7FFF7FFF)
                        ul = pltpu.bitcast(u << 16, f32)
                        u = pltpu.bitcast(u, f32)
                        mh = u if mh is None else jnp.maximum(mh, u)
                        ml = ul if ml is None else jnp.maximum(ml, ul)
                        if 2 * r < _WSUB:
                            s2 = ul * ul
                            ss = s2 if ss is None else ss + s2
            return jnp.maximum(mh, ml), ss

        x_q = lambda q: xbuf[(1,) + quads0[q]]
        xt_copy.wait()
        ssv, maxv = x_stats(xbuf[1, top0].astype(f32), (None,) * nc, None)
        wq_copy[3].wait()
        M5 = product(0, 4, x_q, None, True)
        b_copy.wait()
        xb_copy.wait()
        bb = b_raw[...].astype(f32)
        for k in range(L):
            bf_ref[k] = bb[k:k + 1, :]
        ssv, maxv = x_stats(xbuf[1, bot0].astype(f32), ssv, maxv)
        wq_copy[0].wait()
        M2 = product(0, 1, x_q, None, True)
        M1 = product(0, 0, x_q, None, True)
        wq_copy[1].wait()
        wq_copy[2].wait()
        b1, b2 = bias(0, m0)
        M3b = product(0, 2, x_q, b2, True, True)
        M4b = product(0, 3, x_q, b1, True, True)
        C11 = product(0, 6, x_q, M1 + M4b - M5, True)
        C22 = product(0, 5, x_q, M1 + M3b - M2, True)
        for q, C in enumerate((C11, M3b + M5, M2 + M4b, C22)):
            a = x_q(q).astype(f32)
            xs_ref[quads0[q]] = a * C + a

        def first_body(l, carry):
            w_copy(l).wait()
            A = [xs_ref[quads0[q]] for q in range(4)]
            geta = lambda q: A[q]
            b1, b2 = bias(l, m0)
            M5 = product(l, 4, geta, None, True)
            M2 = product(l, 1, geta, None, True)
            M3b = product(l, 2, geta, b2, True, True)
            M4b = product(l, 3, geta, b1, True, True)
            M1 = product(l, 0, geta, None, True)
            C11 = product(l, 6, geta, M1 + M4b - M5, True)
            C22 = product(l, 5, geta, M1 + M3b - M2, True)
            for q, C in enumerate((C11, M3b + M5, M2 + M4b, C22)):
                xs_ref[quads0[q]] = x_q(q).astype(f32) * C + A[q]
            return carry

        lax.fori_loop(1, L, first_body, 0)
        obuf[1, :tm0] = xs_ref[...].astype(bf16)
        pltpu.make_async_copy(obuf.at[1, pl.ds(0, tm0)], o_hbm.at[pl.ds(0, tm0)], osem.at[1]).start()

        def step(i, carry):
            wcar, maxv = carry
            slot = i % 2

            @pl.when(i + 1 < n)
            def _():
                x_copy(i + 1, 1 - slot).start()

            x_copy(i, slot).wait()

            @pl.when(i == 1)
            def _():
                o_wait(tm0, 1)

            @pl.when(i >= 2)
            def _():
                o_wait(tm, slot)

            Xb = [xbuf[(slot,) + quads[q]] for q in range(4)]
            X = [v.astype(f32) for v in Xb]

            mq = []
            for blk in X:
                mx = None
                for c in range(0, h, 128):
                    for r in range(0, m, 8):
                        t = jnp.abs(blk[r:r + 8, c:c + 128])
                        mx = t if mx is None else jnp.maximum(mx, t)
                mq.append(mx)
            t = functools.reduce(jnp.maximum, mq)
            maxv = jnp.maximum(maxv, t * t)
            lw = jnp.minimum(i, L - 1)
            pm, ps = w_stats(lw)
            wcar = tuple((jnp.where(lw == k, pm, a), jnp.where(lw == k, ps, b))
                         for k, (a, b) in enumerate(wcar))

            A = X
            for l in range(L):
                src = Xb if l == 0 else A
                b1, b2 = bias(l, m)
                C = _chain(lambda j, acc: product(l, j, lambda q: src[q], acc, False, j == 3),
                           (b1, b2, b1, b2), True)
                A = [x * c + a for x, c, a in zip(X, C, A)]
            s11 = _split(A[0])
            vals = [A[2], A[3], A[1], s11[2], s11[3], s11[1], s11[0]]
            for v, rc, cp in zip(vals, pieces(quads), o_copies(tm0 + i * tm, slot)):
                obuf[(slot,) + rc] = v.astype(bf16)
                cp.start()
            return wcar, maxv

        z = jnp.zeros((8, 128), f32)
        wcar, maxv = lax.fori_loop(0, n, step, (((z, z),) * L, maxv))

        def unsafe(mx, ms, t):
            ok = jnp.logical_and(mx <= (t * t) * ms, jnp.logical_and(mx < 1e30, ms > 1e-30))
            return jnp.where(ok, 0, 1).astype(jnp.int32)

        cols = functools.reduce(jnp.minimum, [jnp.sum(v, axis=0, keepdims=True) for v in ssv])
        mx_x = jnp.max(maxv)
        bad = unsafe(mx_x, jnp.min(cols) * (1.0 / tm0), _TX)
        gain = 0.0
        for l in range(L):
            mx = jnp.max(wcar[l][0])
            ms = jnp.sum(wcar[l][1]) * (2.0 / (len(_STAT_LEAVES) * _WSUB * g))
            bad = bad + unsafe(mx * mx, ms, _TW)
            gain = gain + jnp.minimum((0.5 * D) * mx_x * ms, 1.0)
        bad = bad + jnp.where(gain <= _GMAX, 0, 1).astype(jnp.int32)

        for t in (n - 2, n - 1):
            o_wait(tm, t % 2)

        @pl.when(bad > 0)
        def _():
            def redo(c, carry):
                rows = pl.ds(pl.multiple_of(c * sc, sc), sc)
                cin = pltpu.make_async_copy(x0_hbm.at[rows], xbuf.at[0, pl.ds(0, sc)], xsem.at[0])
                cin.start()
                cin.wait()

                def body(l, carry):
                    x0c = xbuf[0, :sc, :].astype(f32)
                    x = jnp.where(l == 0, x0c, xs_ref[:sc, :])
                    xn = x0c * (dot(x, w_raw[l]) + bf_ref[l]) + x
                    xs_ref[:sc, :] = xn
                    obuf[0, :sc, :] = xn.astype(bf16)
                    return carry

                lax.fori_loop(0, L, body, 0)
                cout = pltpu.make_async_copy(obuf.at[0, pl.ds(0, sc)], o_hbm.at[rows], osem.at[0])
                cout.start()
                cout.wait()
                return carry

            lax.fori_loop(0, B // sc, redo, 0)

    return pl.pallas_call(
        kernel,
        in_specs=[pl.BlockSpec(memory_space=pl.ANY)] * 3,
        out_specs=pl.BlockSpec(memory_space=pl.ANY),
        out_shape=jax.ShapeDtypeStruct((B, D), x0.dtype),
        scratch_shapes=[
            pltpu.VMEM((L, D, D), bf16),
            pltpu.VMEM((L, len(_SLOT), g // 2, g), jnp.uint32),
            pltpu.VMEM((2, max(tm0, tm), D), bf16),
            pltpu.VMEM((2, max(tm0, tm), D), bf16),
            pltpu.VMEM((tm0, D), f32),
            pltpu.VMEM((L, D), bf16),
            pltpu.VMEM((L, 1, D), f32),
            pltpu.SemaphoreType.DMA((L,)),
            pltpu.SemaphoreType.DMA((2,)),
            pltpu.SemaphoreType.DMA((2,)),
            pltpu.SemaphoreType.DMA((7,)),
        ],
        compiler_params=pltpu.CompilerParams(
            vmem_limit_bytes=120 * 1024 * 1024,
            disable_bounds_checks=True,
        ),
    )(x0, ws, bs)
```

```python
import functools

import jax
import jax.numpy as jnp
from jax import lax
import jax.experimental.pallas as pl
import jax.experimental.pallas.tpu as pltpu

bf16 = jnp.bfloat16
f32 = jnp.float32

_A_OPS = {0: ((0, 1), (3, 1)), 1: ((2, 1), (3, 1)), 2: ((0, 1),), 3: ((3, 1),),
          4: ((0, 1), (1, 1)), 5: ((2, 1), (0, -1)), 6: ((1, 1), (3, -1))}
_B_OPS = {0: ((0, 1), (3, 1)), 1: ((0, 1),), 2: ((1, 1), (3, -1)), 3: ((2, 1), (0, -1)),
          4: ((3, 1),), 5: ((0, 1), (1, 1)), 6: ((2, 1), (3, 1))}
_SWAP = (0, 2, 3)
_SLOT = {k: i for i, k in enumerate((j, j2) for j in range(7) for j2 in range(7)
                                    if len(_B_OPS[j]) * len(_B_OPS[j2]) > 1)}
_STAT_LEAVES = [(j, j2) for j in (2, 3, 5, 6) for j2 in (1, 4)]

_TM0 = 640
_TM = 576
_SC = 128
_WSUB = 32
_TX = 7.0
_TW = 6.5
_GMAX = 2.0


def _split(a):
    r, c = a.shape[0] // 2, a.shape[1] // 2
    return a[:r, :c], a[:r, c:], a[r:, :c], a[r:, c:]


def _join(c11, c12, c21, c22):
    return jnp.concatenate([jnp.concatenate([c11, c12], axis=1),
                            jnp.concatenate([c21, c22], axis=1)], axis=0)


def _lin(terms):
    terms = sorted(terms, key=lambda t: -t[1])
    acc = terms[0][0]
    for v, s in terms[1:]:
        acc = acc + v if s > 0 else acc - v
    return acc


def _lin2(get, o1, o2):
    if len(o1) == 2 and len(o2) == 2:
        t = lambda i, k: (get(o1[i][0], o2[k][0]), o1[i][1] * o2[k][1])
        p1, p2 = [t(0, 0), t(1, 1)], [t(0, 1), t(1, 0)]
        if p2[0][1] > 0 or p2[1][1] > 0:
            return _lin(p1) + _lin(p2)
        return _lin(p1) - _lin([(v, -s) for v, s in p2])
    return _lin([(get(q, q2), s * s2) for q, s in o1 for q2, s2 in o2])


def _chain(mul, acc, same, alt=False):
    a11, a12, a21, a22 = (None,) * 4 if acc is None else acc
    if alt:
        r1 = mul(1, a21)
        r2 = mul(3, r1)
        r3 = mul(0, -r1 if a21 is None else a21 - r1)
    else:
        r1 = mul(3, a21)
        r2 = mul(1, r1)
        r3 = mul(0, r1 - r2)
    if acc is None:
        r4 = mul(5, r3)
        r5 = mul(2, r4)
        f = r5 - r4
        r6 = mul(4, f)
        r7 = mul(6, (r3 + r2) + (f - r6))
    elif same:
        r4 = mul(5, r3)
        r5 = mul(2, r4 + a22)
        f = r5 - r4
        r6 = mul(4, f)
        r7 = mul(6, (r3 + r2) + (f - r6))
    else:
        r4 = mul(5, r3 + a22)
        r5 = mul(2, r4)
        f = (r5 - r4) + a12
        r6 = mul(4, f)
        r7 = mul(6, ((r3 + r2) + (a11 - a21)) + (f - r6))
    return r7, r6, r2, r5


@jax.jit
def pallas_standalone__dcn_v2_cross__recsys_kernel(
    x0: jax.Array,
    ws: jax.Array,
    bs: jax.Array,
):
    B, D = x0.shape
    L = ws.shape[0]
    tm0, tm, sc = _TM0, _TM, _SC
    h, g, nc = D // 2, D // 4, D // 128
    n = (B - tm0) // tm
    assert tm0 + n * tm == B and n >= max(L, 2) and B % sc == 0 and D % 512 == 0
    m0, m = tm0 // 2, tm // 2

    def kernel(x0_hbm, w_hbm, b_hbm, o_hbm, w_raw, s2_w, xbuf, obuf, xs_ref, xf_ref, b_raw, bf_ref,
               wsem, xsem, osem, psem):
        lo, hi = slice(0, h), slice(h, D)
        wq = [(lo, lo), (lo, hi), (hi, lo), (hi, hi)]

        def quads_of(t):
            top, bot = slice(0, t // 2), slice(t // 2, t)
            return [(top, lo), (top, hi), (bot, lo), (bot, hi)]

        quads0, quads = quads_of(tm0), quads_of(tm)
        top0, bot0 = slice(0, m0), slice(m0, tm0)

        def x_copy(i, slot):
            return pltpu.make_async_copy(x0_hbm.at[pl.ds(tm0 + i * tm, tm)],
                                         xbuf.at[slot, pl.ds(0, tm)], xsem.at[slot])

        def pieces(qs):
            r, c = qs[0]
            rm, cm = (r.start + r.stop) // 2, (c.start + c.stop) // 2
            rt, rb, cl, cr = slice(r.start, rm), slice(rm, r.stop), slice(c.start, cm), slice(cm, c.stop)
            return [qs[2], qs[3], qs[1], (rb, cl), (rb, cr), (rt, cr), (rt, cl)]

        def o_copies(row0, slot):
            return [pltpu.make_async_copy(obuf.at[slot, r, c],
                                          o_hbm.at[pl.ds(row0 + r.start, r.stop - r.start), c],
                                          osem.at[slot]) for r, c in pieces(quads)]

        def o_wait(rows, slot):
            v = obuf.at[slot, pl.ds(0, rows)]
            pltpu.make_async_copy(v, v, osem.at[slot]).wait()

        def w_copy(l):
            return pltpu.make_async_copy(w_hbm.at[l], w_raw.at[l], wsem.at[l])

        b_copy = pltpu.make_async_copy(b_hbm, b_raw, psem.at[0])
        wq_copy = [pltpu.make_async_copy(w_hbm.at[(0,) + wq[q]], w_raw.at[(0,) + wq[q]], psem.at[1 + q])
                   for q in range(4)]
        xt_copy = pltpu.make_async_copy(x0_hbm.at[top0], xbuf.at[1, top0], psem.at[5])
        xb_copy = pltpu.make_async_copy(x0_hbm.at[bot0], xbuf.at[1, bot0], psem.at[6])

        copies = [xt_copy, wq_copy[3], b_copy, xb_copy, wq_copy[0], wq_copy[1], wq_copy[2]]
        copies += [w_copy(l) for l in range(1, L)] + [x_copy(0, 0)]

        def issue(k, carry):
            for idx, cp in enumerate(copies):
                @pl.when(k == idx)
                def _(cp=cp):
                    cp.start()
            return carry

        lax.fori_loop(0, len(copies), issue, 0)

        def dot(a, w):
            return jnp.dot(a.astype(bf16), w, preferred_element_type=f32)

        def raw_sub(l, j, q, q2):
            c2 = (q2 % 2) ^ (1 if j in _SWAP else 0)
            rr = (q // 2) * h + (q2 // 2) * g
            cc = (q % 2) * h + c2 * g
            return w_raw[l, rr:rr + g, cc:cc + g]

        def product(l, j, geta, acc, build, isbias=False):
            sub = lambda q, q2: _split(geta(q))[q2]
            if build and len(_B_OPS[j]) > 1:
                V = [_lin([(raw_sub(l, j, q, q2).astype(f32), s) for q, s in _B_OPS[j]])
                     for q2 in range(4)]

            def mul2(j2, acc2):
                o1, o2 = _A_OPS[j], _A_OPS[j2]
                if len(o1) * len(o2) == 1:
                    a2 = sub(o1[0][0], o2[0][0])
                else:
                    a2 = _lin2(lambda q, q2: sub(q, q2).astype(f32), o1, o2)
                if (j, j2) not in _SLOT:
                    w = raw_sub(l, j, _B_OPS[j][0][0], _B_OPS[j2][0][0])
                elif not build:
                    w = pltpu.bitcast(s2_w[l, _SLOT[j, j2]], bf16)
                else:
                    if len(_B_OPS[j]) > 1:
                        wf = _lin([(V[q2], s) for q2, s in _B_OPS[j2]])
                    else:
                        wf = _lin([(raw_sub(l, j, _B_OPS[j][0][0], q2).astype(f32), s)
                                   for q2, s in _B_OPS[j2]])
                    w = wf.astype(bf16)
                    s2_w[l, _SLOT[j, j2]] = pltpu.bitcast(w, jnp.uint32)
                r = dot(a2, w)
                return r if acc2 is None else r + acc2

            a = None if acc is None else _split(acc)
            if j in _SWAP:
                c = _chain(mul2, None if a is None else (a[1], a[0], a[3], a[2]), isbias, build)
                return _join(c[1], c[0], c[3], c[2])
            return _join(*_chain(mul2, a, isbias, build))

        def bias(l, rows):
            bv = bf_ref[l]
            return jnp.broadcast_to(bv[:, lo], (rows, h)), jnp.broadcast_to(bv[:, hi], (rows, h))

        def x_stats(blk, ssv, maxv):
            ssv = list(ssv)
            for c in range(nc):
                ss = mx = None
                for r in range(0, blk.shape[0], 8):
                    t = blk[r:r + 8, c * 128:(c + 1) * 128]
                    t = t * t
                    ss = t if ss is None else ss + t
                    mx = t if mx is None else jnp.maximum(mx, t)
                ssv[c] = ss if ssv[c] is None else ssv[c] + ss
                maxv = mx if maxv is None else jnp.maximum(maxv, mx)
            return tuple(ssv), maxv

        def w_stats(l):
            mh = ml = ss = None
            for key in _STAT_LEAVES:
                wv = pltpu.bitcast(s2_w[l, _SLOT[key]], jnp.int32)
                for r in range(0, g // 2, 8):
                    for c in range(0, g, 128):
                        u = wv[r:r + 8, c:c + 128] & jnp.int32(0x7FFF7FFF)
                        ul = pltpu.bitcast(u << 16, f32)
                        u = pltpu.bitcast(u, f32)
                        mh = u if mh is None else jnp.maximum(mh, u)
                        ml = ul if ml is None else jnp.maximum(ml, ul)
                        if 2 * r < _WSUB:
                            s2 = ul * ul
                            ss = s2 if ss is None else ss + s2
            return jnp.maximum(mh, ml), ss

        x_q = lambda q: xf_ref[quads0[q]]
        xt_copy.wait()
        xt = xbuf[1, top0].astype(f32)
        xf_ref[top0] = xt
        ssv, maxv = x_stats(xt, (None,) * nc, None)
        wq_copy[3].wait()
        M5 = product(0, 4, x_q, None, True)
        b_copy.wait()
        xb_copy.wait()
        bb = b_raw[...].astype(f32)
        for k in range(L):
            bf_ref[k] = bb[k:k + 1, :]
        xb = xbuf[1, bot0].astype(f32)
        xf_ref[bot0] = xb
        ssv, maxv = x_stats(xb, ssv, maxv)
        wq_copy[0].wait()
        M2 = product(0, 1, x_q, None, True)
        M1 = product(0, 0, x_q, None, True)
        wq_copy[1].wait()
        wq_copy[2].wait()
        b1, b2 = bias(0, m0)
        M3b = product(0, 2, x_q, b2, True, True)
        M4b = product(0, 3, x_q, b1, True, True)
        C11 = product(0, 6, x_q, M1 + M4b - M5, True)
        C22 = product(0, 5, x_q, M1 + M3b - M2, True)
        for q, C in enumerate((C11, M3b + M5, M2 + M4b, C22)):
            a = x_q(q)
            xs_ref[quads0[q]] = a * C + a

        def first_body(l, carry):
            w_copy(l).wait()
            A = [xs_ref[quads0[q]] for q in range(4)]
            geta = lambda q: A[q]
            b1, b2 = bias(l, m0)
            M2 = product(l, 1, geta, None, True)
            M7 = product(l, 6, geta, None, True)
            T22 = product(l, 5, geta, -M2, True)
            M4b = product(l, 3, geta, b1, True, True)
            M1 = product(l, 0, geta, None, True)
            M3b = product(l, 2, geta, b2, True, True)
            P = ((M7 + M4b) + M1) + M3b
            C12 = product(l, 4, geta, M3b, True)
            for q, C in enumerate((P - C12, C12, M2 + M4b, (T22 + M1) + M3b)):
                xs_ref[quads0[q]] = x_q(q) * C + A[q]
            return carry

        lax.fori_loop(1, L, first_body, 0)
        obuf[1, :tm0] = xs_ref[...].astype(bf16)
        pltpu.make_async_copy(obuf.at[1, pl.ds(0, tm0)], o_hbm.at[pl.ds(0, tm0)], osem.at[1]).start()

        def step(i, carry):
            wcar, maxv = carry
            slot = i % 2

            @pl.when(i + 1 < n)
            def _():
                x_copy(i + 1, 1 - slot).start()

            x_copy(i, slot).wait()

            @pl.when(i == 1)
            def _():
                o_wait(tm0, 1)

            @pl.when(i >= 2)
            def _():
                o_wait(tm, slot)

            Xb = [xbuf[(slot,) + quads[q]] for q in range(4)]
            X = [v.astype(f32) for v in Xb]

            mq = []
            for blk in X:
                mx = None
                for c in range(0, h, 128):
                    for r in range(0, m, 8):
                        t = jnp.abs(blk[r:r + 8, c:c + 128])
                        mx = t if mx is None else jnp.maximum(mx, t)
                mq.append(mx)
            t = functools.reduce(jnp.maximum, mq)
            maxv = jnp.maximum(maxv, t * t)
            lw = jnp.minimum(i, L - 1)
            pm, ps = w_stats(lw)
            wcar = tuple((jnp.where(lw == k, pm, a), jnp.where(lw == k, ps, b))
                         for k, (a, b) in enumerate(wcar))

            A = X
            for l in range(L):
                src = Xb if l == 0 else A
                b1, b2 = bias(l, m)
                C = _chain(lambda j, acc: product(l, j, lambda q: src[q], acc, False, j == 3),
                           (b1, b2, b1, b2), True)
                A = [x * c + a for x, c, a in zip(X, C, A)]
            s11 = _split(A[0])
            vals = [A[2], A[3], A[1], s11[2], s11[3], s11[1], s11[0]]
            for v, rc, cp in zip(vals, pieces(quads), o_copies(tm0 + i * tm, slot)):
                obuf[(slot,) + rc] = v.astype(bf16)
                cp.start()
            return wcar, maxv

        z = jnp.zeros((8, 128), f32)
        wcar, maxv = lax.fori_loop(0, n, step, (((z, z),) * L, maxv))

        def unsafe(mx, ms, t):
            ok = jnp.logical_and(mx <= (t * t) * ms, jnp.logical_and(mx < 1e30, ms > 1e-30))
            return jnp.where(ok, 0, 1).astype(jnp.int32)

        cols = functools.reduce(jnp.minimum, [jnp.sum(v, axis=0, keepdims=True) for v in ssv])
        mx_x = jnp.max(maxv)
        bad = unsafe(mx_x, jnp.min(cols) * (1.0 / tm0), _TX)
        gain = 0.0
        for l in range(L):
            mx = jnp.max(wcar[l][0])
            ms = jnp.sum(wcar[l][1]) * (2.0 / (len(_STAT_LEAVES) * _WSUB * g))
            bad = bad + unsafe(mx * mx, ms, _TW)
            gain = gain + jnp.minimum((0.5 * D) * mx_x * ms, 1.0)
        bad = bad + jnp.where(gain <= _GMAX, 0, 1).astype(jnp.int32)

        for t in (n - 2, n - 1):
            o_wait(tm, t % 2)

        @pl.when(bad > 0)
        def _():
            def redo(c, carry):
                rows = pl.ds(pl.multiple_of(c * sc, sc), sc)
                cin = pltpu.make_async_copy(x0_hbm.at[rows], xbuf.at[0, pl.ds(0, sc)], xsem.at[0])
                cin.start()
                cin.wait()

                def body(l, carry):
                    x0c = xbuf[0, :sc, :].astype(f32)
                    x = jnp.where(l == 0, x0c, xs_ref[:sc, :])
                    xn = x0c * (dot(x, w_raw[l]) + bf_ref[l]) + x
                    xs_ref[:sc, :] = xn
                    obuf[0, :sc, :] = xn.astype(bf16)
                    return carry

                lax.fori_loop(0, L, body, 0)
                cout = pltpu.make_async_copy(obuf.at[0, pl.ds(0, sc)], o_hbm.at[rows], osem.at[0])
                cout.start()
                cout.wait()
                return carry

            lax.fori_loop(0, B // sc, redo, 0)

    return pl.pallas_call(
        kernel,
        in_specs=[pl.BlockSpec(memory_space=pl.ANY)] * 3,
        out_specs=pl.BlockSpec(memory_space=pl.ANY),
        out_shape=jax.ShapeDtypeStruct((B, D), x0.dtype),
        scratch_shapes=[
            pltpu.VMEM((L, D, D), bf16),
            pltpu.VMEM((L, len(_SLOT), g // 2, g), jnp.uint32),
            pltpu.VMEM((2, max(tm0, tm), D), bf16),
            pltpu.VMEM((2, max(tm0, tm), D), bf16),
            pltpu.VMEM((tm0, D), f32),
            pltpu.VMEM((tm0, D), f32),
            pltpu.VMEM((L, D), bf16),
            pltpu.VMEM((L, 1, D), f32),
            pltpu.SemaphoreType.DMA((L,)),
            pltpu.SemaphoreType.DMA((2,)),
            pltpu.SemaphoreType.DMA((2,)),
            pltpu.SemaphoreType.DMA((7,)),
        ],
        compiler_params=pltpu.CompilerParams(
            vmem_limit_bytes=96 * 1024 * 1024,
            disable_bounds_checks=True,
        ),
    )(x0, ws, bs)
```
